```python
import os as _os
_os.environ.setdefault("JAX_PLATFORMS", "cpu")
import jax
import jax.numpy as jnp

def _softmax(x, axis=-1):
    return jax.nn.softmax(x, axis=axis)
def _gelu(x):
    return jax.nn.gelu(x, approximate=True)
def _silu(x):
    return jax.nn.silu(x)
def _sigmoid(x):
    return jax.nn.sigmoid(x)
def _layernorm(x, axis=-1, eps=1e-5):
    m = jnp.mean(x, axis=axis, keepdims=True)
    v = jnp.var(x, axis=axis, keepdims=True)
    return (x - m) / jnp.sqrt(v + eps)
def _scatter_add(tgt, idx, src, axis=0):
    return tgt.at[idx].add(src)
def _segment_sum(src, seg, n):
    return jax.ops.segment_sum(src, seg, n)
class _Rng:
    def __init__(self, key):
        self._k = key
    def _next(self):
        self._k, sub = jax.random.split(self._k)
        return sub
    def normal(self, shape):
        return jax.random.normal(self._next(), shape, dtype=jnp.bfloat16)
    def randint(self, lo, hi, shape):
        return jax.random.randint(self._next(), shape, lo, hi, dtype=jnp.int32)
    def uniform(self, shape, lo=0.0, hi=1.0):
        return jax.random.uniform(self._next(), shape, jnp.bfloat16, lo, hi)
    def permutation(self, n):
        return jax.random.permutation(self._next(), n)


kernel_name = 'concat_heads__grouped_kv_mqa__sliding_block__prompt'

def setup_inputs():
    _rng = _Rng(jax.random.key(int.from_bytes(__import__("os").urandom(4), "little")))
    _w = (lambda a: (lambda t: t.astype(jnp.bfloat16) if jnp.issubdtype(t.dtype, jnp.floating) else t)(jnp.asarray(a)))
    def _A_setup():
        B, S, D, H = 1, 2048, 1024, 32
        Dh = D // H
        return {
            "x": _w((lambda *s: _rng.normal(s) * 0.05)(B, S, D)),
            "wq": _w((lambda *s: _rng.normal(s) * 1.6)(D, H * Dh)),
            "wk": _w((lambda *s: _rng.normal(s) * 1.6)(D, Dh)),
            "wv": _w((lambda *s: _rng.normal(s) * 0.1)(D, Dh)),
            "wo": _w((lambda *s: _rng.normal(s) * 0.1)(H * Dh, D)),
        }
    _A_in = _A_setup()

    def _B_setup():
        B, S, D = 1, 2048, 1024
        return {
            "x": _w((lambda *s: _rng.normal(s) * 0.2)(B, S, D)),
            "wqkv": _w((lambda *s: _rng.normal(s) * 0.2)(D, 3 * D)),
            "wo": _w((lambda *s: _rng.normal(s) * 0.05)(D, D)),
        }
    _B_in = _B_setup()

    return {
        "A_x": _A_in["x"],
        "A_wq": _A_in["wq"],
        "A_wk": _A_in["wk"],
        "A_wv": _A_in["wv"],
        "A_wo": _A_in["wo"],
        "B_x": _B_in["x"],
        "B_wqkv": _B_in["wqkv"],
        "B_wo": _B_in["wo"],
    }

def reference(A_x, A_wq, A_wk, A_wv, A_wo, B_x, B_wqkv, B_wo):
    def _A_ref(x, wq, wk, wv, wo):
        B, S, D = x.shape
        H = 32
        Dh = D // H
        q = (lambda x, *d: x.transpose(*d))((x @ wq).reshape(B, S, H, Dh), 0, 2, 1, 3)
        k = x @ wk
        v = x @ wv
        scores = jnp.einsum("bhqd,bkd->bhqk", q, k) * (Dh ** -0.5)
        p = _softmax(scores, axis=-1)
        o = jnp.einsum("bhqk,bkd->bhqd", p, v)
        return (lambda x, *d: x.transpose(*d))(o, 0, 2, 1, 3).reshape(B, S, H * Dh) @ wo

    def _B_ref(x, wqkv, wo):
        B, S, D = x.shape
        H = 32; Dh = D // H; W = 256
        qkv = (lambda x, *d: x.transpose(*d))((x @ wqkv).reshape(B, S, 3, H, Dh), 2, 0, 3, 1, 4)
        q, k, v = qkv[0], qkv[1], qkv[2]
        scores = jnp.einsum("bhqd,bhkd->bhqk", q, k) * (Dh ** -0.5)
        idx = jnp.arange(S)
        mask = (idx[:, None] - idx[None, :] >= 0) & (idx[:, None] - idx[None, :] < W)
        scores = jnp.where(mask[None, None], scores, -1e9)
        p = _softmax(scores, axis=-1)
        o = jnp.einsum("bhqk,bhkd->bhqd", p, v)
        return (lambda x, *d: x.transpose(*d))(o, 0, 2, 1, 3).reshape(B, S, D) @ wo

    a = _A_ref(A_x, A_wq, A_wk, A_wv, A_wo)
    b = _B_ref(B_x, B_wqkv, B_wo)
    return jnp.concatenate([a, b], axis=-1)
```

```python
import jax
import jax.numpy as jnp
from jax import lax
import jax.experimental.pallas as pl
import jax.experimental.pallas.tpu as pltpu

S = 2048
D = 1024
H = 32
DH = D // H
W = 256
LOG2E = 1.4426950408889634
QSCALE = (DH ** -0.5) * LOG2E
NEG = -1e9 * LOG2E

TQ = 512
RK = 128
PAD = W
SROWS = 3 * 128 * 8

BF = jnp.bfloat16
U32 = jnp.uint32
F32 = jnp.float32
NT = (((1,), (1,)), ((), ()))
TN = (((0,), (0,)), ((), ()))


def _tree(xs, op):
    xs = list(xs)
    while len(xs) > 1:
        nx = [op(xs[i], xs[i + 1]) for i in range(0, len(xs) - 1, 2)]
        if len(xs) % 2:
            nx.append(xs[-1])
        xs = nx
    return xs[0]


def _red8(x, op):
    n = x.shape[0] // 8
    x = x.reshape(n, 8, x.shape[1])
    return _tree([x[i] for i in range(n)], op)


def _pack(x_bf16):
    return pltpu.bitcast(x_bf16, U32)


def _unpack(x_u32):
    return pltpu.bitcast(x_u32, BF)


def _kernel(
    ax_hbm, awq_hbm, awk_hbm, awv_hbm, awo_hbm, bx_hbm, bwqkv_hbm, bwo_hbm,
    out_hbm,
    x_v, wq_v, wk_v, wv_v, wo_a, bx_v, bwqkv_v, wo_b,
    wt_v, wt2_v, qt_v, ka_v, vta_v, kb_v, vtb_v, ot_v, stage_v, m_v, s_a, s_b,
    in_sem, out_sem,
):
    def in_copy(i):
        srcs = [
            (awq_hbm, wq_v), (awk_hbm, wk_v), (awv_hbm, wv_v),
            (ax_hbm.at[pl.ds(0, 512)], x_v.at[pl.ds(0, 512)]),
            (ax_hbm.at[pl.ds(512, 512)], x_v.at[pl.ds(512, 512)]),
            (ax_hbm.at[pl.ds(1024, 512)], x_v.at[pl.ds(1024, 512)]),
            (ax_hbm.at[pl.ds(1536, 512)], x_v.at[pl.ds(1536, 512)]),
            (awo_hbm, wo_a), (bwqkv_hbm, bwqkv_v), (bx_hbm, bx_v), (bwo_hbm, wo_b),
        ]
        src, dst = srcs[i]
        return pltpu.make_async_copy(src, dst, in_sem.at[i])

    def out_copy(slot, qb, half):
        return pltpu.make_async_copy(
            stage_v.at[slot],
            out_hbm.at[pl.ds(pl.multiple_of(qb * 512, 512), 512), pl.ds(half * D, D)],
            out_sem.at[slot],
        )

    for i in range(8):
        in_copy(i).start()

    in_copy(0).wait()
    for c in range(4):
        wt_v[c * 256:(c + 1) * 256, :] = wq_v[:, c * 256:(c + 1) * 256].T
    in_copy(1).wait()
    in_copy(2).wait()
    wkv = jnp.concatenate(
        [wk_v[...], wv_v[...], jnp.zeros((D, 128 - 2 * DH), BF)], axis=1)
    wt_v[D:D + 64, :] = wkv.T[0:64, :]

    for c in range(4):
        in_copy(3 + c).wait()
        xc = x_v[c * 512:(c + 1) * 512, :]
        r = lax.dot_general(wt_v[0:D + 64, :], xc, NT, preferred_element_type=F32)
        qt_v[:, c * 512:(c + 1) * 512] = _pack((r[0:D] * QSCALE).astype(BF))
        kv = jnp.concatenate([r[D:D + 64], jnp.zeros((64, 512), F32)], axis=0)
        ka_v[c * 256:(c + 1) * 256, :] = _pack(kv.T.astype(BF))
        vta_v[:, c * 512:(c + 1) * 512] = _pack(r[D + 32:D + 64].astype(BF))

    for i in range(8, 11):
        in_copy(i).start()

    def a_qtile(t):
        h = lax.rem(t, H)
        qb = t // H
        return qt_v[pl.ds(pl.multiple_of(h * 16, 16), 16),
                    pl.ds(pl.multiple_of(qb * TQ, TQ), TQ)]

    def a_s1_round(qt, s_dst, j):
        kk = _unpack(ka_v[j * RK // 2:(j + 1) * RK // 2, :])
        s = jnp.dot(kk[:, 0:DH], qt, preferred_element_type=F32)
        s_dst[j * RK:(j + 1) * RK, :] = s
        return _red8(s, jnp.maximum)

    def a_s2_round(s_src, j, mb):
        s = s_src[j * RK:(j + 1) * RK, :]
        p = jnp.exp2(s.reshape(RK // 8, 8, TQ) - mb[None]).reshape(RK, TQ)
        lj = _red8(p, jnp.add)
        vt = _unpack(vta_v[:, j * RK:(j + 1) * RK])
        pv = jnp.dot(vt, p.astype(BF), preferred_element_type=F32)
        return lj, pv

    def a_slot(t, s_src, s_dst):
        mb = m_v[0:8, :]
        qt = _unpack(a_qtile(jnp.minimum(t + 1, H * (S // TQ) - 1)))
        m = l = acc = None
        for j in range(S // RK):
            mj = a_s1_round(qt, s_dst, j)
            m = mj if m is None else jnp.maximum(m, mj)
            lj, pv = a_s2_round(s_src, j, mb)
            l = lj if l is None else l + lj
            acc = pv if acc is None else acc + pv
        m_v[0:8, :] = jnp.broadcast_to(jnp.max(m, axis=0, keepdims=True), (8, TQ))
        l = jnp.sum(l, axis=0, keepdims=True)
        h = lax.rem(t, H)
        ot_v[pl.ds(pl.multiple_of(h * 16, 16), 16), 0:TQ] = _pack((acc * (1.0 / l)).astype(BF))

    def out_proj(w_ref, col0, slot):
        ot = _unpack(ot_v[:, pl.ds(col0, 512)])
        r = lax.dot_general(ot, w_ref[...], TN, preferred_element_type=F32)
        stage_v[slot] = r.astype(BF)

    qt0 = _unpack(qt_v[0:16, 0:TQ])
    m0 = None
    for j in range(S // RK):
        mj = a_s1_round(qt0, s_a, j)
        m0 = mj if m0 is None else jnp.maximum(m0, mj)
    m_v[0:8, :] = jnp.broadcast_to(jnp.max(m0, axis=0, keepdims=True), (8, TQ))

    in_copy(7).wait()

    def a_body(t, carry):
        @pl.when(lax.rem(t, 2) == 0)
        def _():
            a_slot(t, s_a, s_b)

        @pl.when(lax.rem(t, 2) == 1)
        def _():
            a_slot(t, s_b, s_a)

        @pl.when(lax.rem(t, H) == H - 1)
        def _():
            qb = t // H
            slot = lax.rem(qb, 2)

            @pl.when(qb >= 2)
            def _():
                out_copy(slot, qb - 2, 0).wait()

            out_proj(wo_a, 0, slot)
            out_copy(slot, qb, 0).start()
        return carry

    lax.fori_loop(0, H * (S // TQ), a_body, 0)

    in_copy(8).wait()
    for c in range(4):
        wt_v[c * 256:(c + 1) * 256, :] = bwqkv_v[:, c * 256:(c + 1) * 256].T
        wt2_v[c * 256:(c + 1) * 256, :] = bwqkv_v[:, 2 * D + c * 256:2 * D + (c + 1) * 256].T
    kb_v[0:PAD // 2, :] = jnp.zeros((PAD // 2, D), U32)
    vtb_v[:, 0:PAD] = jnp.zeros((D // 2, PAD), U32)
    in_copy(9).wait()
    for c in range(4):
        xc = bx_v[c * 512:(c + 1) * 512, :]
        r = lax.dot_general(wt_v[0:D, :], xc, NT, preferred_element_type=F32)
        qt_v[:, c * 512:(c + 1) * 512] = _pack((r * QSCALE).astype(BF))
        r = lax.dot_general(wt2_v[...], xc, NT, preferred_element_type=F32)
        vtb_v[:, PAD + c * 512:PAD + (c + 1) * 512] = _pack(r.astype(BF))
        r = jnp.dot(xc, bwqkv_v[:, D:2 * D], preferred_element_type=F32)
        kb_v[(PAD + c * 512) // 2:(PAD + (c + 1) * 512) // 2, :] = _pack(r.astype(BF))

    ri = lax.broadcasted_iota(jnp.int32, (128, 128), 0)
    ci = lax.broadcasted_iota(jnp.int32, (128, 128), 1)
    NGRP = 8

    class BU1:
        def __init__(self, t, g, s_dst):
            self.t, self.g, self.s_dst = t, g, s_dst
            self.q0 = pl.multiple_of(t * 128, 128)
            q4 = qt_v[g * 64:(g + 1) * 64, pl.ds(self.q0, 128)]
            zz = jnp.zeros((16, 128), U32)
            ws = []
            for h in range(4):
                ws.append(jnp.concatenate(
                    [q4[hh * 16:(hh + 1) * 16] if hh == h else zz for hh in range(4)], axis=0))
            self.w = _unpack(jnp.concatenate(ws, axis=1))
            self.m = None

        def round(self, r):
            t, g = self.t, self.g
            kk = _unpack(kb_v[pl.ds(pl.multiple_of((self.q0 + r * 128) // 2, 64), 64),
                              g * 128:(g + 1) * 128])
            s = jnp.dot(kk, self.w, preferred_element_type=F32)
            if r == 0:
                valid = (ri > ci) & (t >= 2)
            elif r == 1:
                valid = (ri >= 0) & (t >= 1)
            else:
                valid = ri <= ci
            s = jnp.concatenate(
                [jnp.where(valid, s[:, h * 128:(h + 1) * 128], NEG) for h in range(4)], axis=1)
            self.s_dst[g * 384 + r * 128:g * 384 + (r + 1) * 128, :] = s
            mr = _red8(s, jnp.maximum)
            self.m = mr if self.m is None else jnp.maximum(self.m, mr)
            if r == 2:
                m_v[g * 8:(g + 1) * 8, :] = self.m

    class BU2:
        def __init__(self, t, g, s_src, mb):
            self.t, self.g, self.s_src, self.mb = t, g, s_src, mb
            self.q0 = pl.multiple_of(t * 128, 128)
            self.l = None
            self.accs = [None] * 4

        def round(self, r):
            g, q0 = self.g, self.q0
            s = self.s_src[g * 384 + r * 128:g * 384 + (r + 1) * 128, :]
            p = jnp.exp2(s.reshape(16, 8, 512) - self.mb[None]).reshape(128, 512)
            lr = _red8(p, jnp.add)
            self.l = lr if self.l is None else self.l + lr
            for h in range(4):
                pbh = p[:, h * 128:(h + 1) * 128].astype(BF)
                vt = _unpack(vtb_v[g * 64 + h * 16:g * 64 + (h + 1) * 16,
                                   pl.ds(q0 + r * 128, 128)])
                pv = jnp.dot(vt, pbh, preferred_element_type=F32)
                self.accs[h] = pv if self.accs[h] is None else self.accs[h] + pv
            if r == 2:
                rl = 1.0 / jnp.sum(self.l, axis=0, keepdims=True)
                oc = pl.multiple_of(lax.rem(self.t, 4) * 128, 128)
                for h in range(4):
                    ot_v[g * 64 + h * 16:g * 64 + (h + 1) * 16, pl.ds(oc, 128)] = _pack(
                        (self.accs[h] * rl[:, h * 128:(h + 1) * 128]).astype(BF))

    NTB = S // 128

    def b_slot(t, s_src, s_dst):
        tn = jnp.minimum(t + 1, NTB - 1)
        mbs = []
        for g in range(NGRP):
            mm = m_v[g * 8:(g + 1) * 8, :]
            mbs.append(jnp.broadcast_to(jnp.max(mm, axis=0, keepdims=True), (8, 512)))
        for g in range(NGRP):
            b = BU2(t, g, s_src, mbs[g])
            a = BU1(tn, g, s_dst)
            for r in range(3):
                a.round(r)
                b.round(r)

    for g in range(NGRP):
        u = BU1(0, g, s_a)
        for r in range(3):
            u.round(r)

    in_copy(10).wait()

    def b_body(t, carry):
        @pl.when(lax.rem(t, 2) == 0)
        def _():
            b_slot(t, s_a, s_b)

        @pl.when(lax.rem(t, 2) == 1)
        def _():
            b_slot(t, s_b, s_a)

        @pl.when(lax.rem(t, 4) == 3)
        def _():
            qb = t // 4
            slot = lax.rem(qb, 2)

            @pl.when(qb < 2)
            def _():
                out_copy(slot, qb + 2, 0).wait()

            @pl.when(qb >= 2)
            def _():
                out_copy(slot, qb - 2, 1).wait()

            out_proj(wo_b, 0, slot)
            out_copy(slot, qb, 1).start()
        return carry

    lax.fori_loop(0, NTB, b_body, 0)
    out_copy(0, 2, 1).wait()
    out_copy(1, 3, 1).wait()


@jax.jit
def pallas_concat_heads__grouped_kv_mqa__sliding_block__prompt_kernel(
    A_x: jax.Array,
    A_wq: jax.Array,
    A_wk: jax.Array,
    A_wv: jax.Array,
    A_wo: jax.Array,
    B_x: jax.Array,
    B_wqkv: jax.Array,
    B_wo: jax.Array,
):
    B = A_x.shape[0]
    assert B == 1 and A_x.shape == (1, S, D) and B_x.shape == (1, S, D)

    scratch = [
        pltpu.VMEM((S, D), BF),
        pltpu.VMEM((D, D), BF),
        pltpu.VMEM((D, DH), BF),
        pltpu.VMEM((D, DH), BF),
        pltpu.VMEM((D, D), BF),
        pltpu.VMEM((S, D), BF),
        pltpu.VMEM((D, 3 * D), BF),
        pltpu.VMEM((D, D), BF),
        pltpu.VMEM((D + 64, D), BF),
        pltpu.VMEM((D, D), BF),
        pltpu.VMEM((D // 2, S), U32),
        pltpu.VMEM((S // 2, 128), U32),
        pltpu.VMEM((DH // 2, S), U32),
        pltpu.VMEM(((S + PAD) // 2, D), U32),
        pltpu.VMEM((D // 2, S + PAD), U32),
        pltpu.VMEM((D // 2, 512), U32),
        pltpu.VMEM((2, 512, D), BF),
        pltpu.VMEM((64, 512), F32),
        pltpu.VMEM((SROWS, 512), F32),
        pltpu.VMEM((SROWS, 512), F32),
        pltpu.SemaphoreType.DMA((11,)),
        pltpu.SemaphoreType.DMA((2,)),
    ]
    any_spec = pl.BlockSpec(memory_space=pl.ANY)
    out = pl.pallas_call(
        _kernel,
        out_shape=jax.ShapeDtypeStruct((S, 2 * D), BF),
        in_specs=[any_spec] * 8,
        out_specs=any_spec,
        scratch_shapes=scratch,
        compiler_params=pltpu.CompilerParams(vmem_limit_bytes=120 * 1024 * 1024),
    )(A_x.reshape(S, D), A_wq, A_wk, A_wv, A_wo, B_x.reshape(S, D), B_wqkv, B_wo)
    return out.reshape(1, S, 2 * D)
```

```python
import jax
import jax.numpy as jnp
from jax import lax
import jax.experimental.pallas as pl
import jax.experimental.pallas.tpu as pltpu


S = 2048
D = 1024
H = 32
DH = D // H
W = 256
LOG2E = 1.4426950408889634
QSCALE = (DH ** -0.5) * LOG2E
NEG = -1e9 * LOG2E

TQ = 512
RK = 128
SROWS = 3 * 128 * 8
assert W == 256

BF = jnp.bfloat16
U32 = jnp.uint32
F32 = jnp.float32
NT = (((1,), (1,)), ((), ()))
TN = (((0,), (0,)), ((), ()))


def _tree(xs, op):
    xs = list(xs)
    while len(xs) > 1:
        nx = [op(xs[i], xs[i + 1]) for i in range(0, len(xs) - 1, 2)]
        if len(xs) % 2:
            nx.append(xs[-1])
        xs = nx
    return xs[0]


def _red8(x, op):
    n = x.shape[0] // 8
    x = x.reshape(n, 8, x.shape[1])
    return _tree([x[i] for i in range(n)], op)


def _pack(x_bf16):
    return pltpu.bitcast(x_bf16, U32)


def _unpack(x_u32):
    return pltpu.bitcast(x_u32, BF)


def _dep(x, y, zv):
    if y is None:
        return x
    xb = pltpu.bitcast(x, U32)
    yb = pltpu.bitcast(y, U32)
    return pltpu.bitcast(xb | (yb & zv), x.dtype)


def _off(i, mul, add):
    return i * mul + add if isinstance(i, int) else pl.multiple_of(i * mul + add, mul)


def _colmax_b(m):
    return jnp.broadcast_to(jnp.max(m, axis=0, keepdims=True), m.shape)


def _kernel(
    ax_hbm, awq_hbm, awk_hbm, awv_hbm, awo_hbm, bx_hbm, bwqkv_hbm, bwo_hbm,
    out_hbm,
    x_v, wq_v, wo_a, bx_v, bwqkv_v, wo_b,
    wt_v, wtb_v, qt_v, ka_v, vta_v, kb_v, vtb_v, ota_v, otb_v, stage_v, m_v, cap_v,
    s_0, s_1, s_2,
    in_sem, out_sem,
):
    s_bufs = (s_0, s_1, s_2)

    IN = {}
    for c in range(4):
        IN["wq%d" % c] = (awq_hbm.at[:, pl.ds(c * 256, 256)], wq_v.at[:, pl.ds(c * 256, 256)])
        IN["x%d" % c] = (ax_hbm.at[pl.ds(c * 512, 512)], x_v.at[pl.ds(c * 512, 512)])
    IN["wk"] = (awk_hbm, wt_v.at[pl.ds(D, DH)])
    IN["wv"] = (awv_hbm, wt_v.at[pl.ds(D + DH, DH)])
    IN["woa"] = (awo_hbm, wo_a)
    IN["wqkv"] = (bwqkv_hbm, bwqkv_v)
    IN["bx"] = (bx_hbm, bx_v)
    IN["wob"] = (bwo_hbm, wo_b)
    IN_IDX = {k: i for i, k in enumerate(sorted(IN))}

    def in_copy(name):
        src, dst = IN[name]
        return pltpu.make_async_copy(src, dst, in_sem.at[IN_IDX[name]])

    def out_copy(slot, qb, half):
        return pltpu.make_async_copy(
            stage_v.at[slot],
            out_hbm.at[pl.ds(_off(qb, 512, 0), 512), pl.ds(_off(half, D, 0), D)],
            out_sem.at[slot],
        )

    for name in ("wq0", "x0"):
        in_copy(name).start()

    def a_q(c, xc, r0, nr):
        r = lax.dot_general(wt_v[r0:r0 + nr, :], xc, NT, preferred_element_type=F32)
        qt_v[r0 // 2:(r0 + nr) // 2, c * 512:(c + 1) * 512] = _pack((r * QSCALE).astype(BF))

    def a_kv(c, r):
        kv = jnp.concatenate([r, jnp.zeros((64, 512), F32)], axis=0)
        ka_v[pl.ds(_off(c, 256, 0), 256), :] = _pack(kv.T.astype(BF))
        vta_v[:, pl.ds(_off(c, 512, 0), 512)] = _pack(r[32:64].astype(BF))

    in_copy("wq0").wait()
    for name in ("wq1", "wq2", "wq3", "wk", "wv"):
        in_copy(name).start()
    wt_v[0:256, :] = wq_v[:, 0:256].T
    in_copy("x0").wait()
    for name in ("x1", "x2", "x3", "woa"):
        in_copy(name).start()
    xc = x_v[0:512, :]
    for c in range(4):
        if c > 0:
            in_copy("wq%d" % c).wait()
            wt_v[c * 256:(c + 1) * 256, :] = wq_v[:, c * 256:(c + 1) * 256].T
        if c < 3:
            a_q(0, xc, c * 256, 256)
    in_copy("wk").wait()
    in_copy("wv").wait()
    r = lax.dot_general(wt_v[768:D + 64, :], xc, NT, preferred_element_type=F32)
    qt_v[384:512, 0:512] = _pack((r[0:256] * QSCALE).astype(BF))
    a_kv(0, r[256:320])
    for c in range(1, 4):
        in_copy("x%d" % c).wait()

    def a_proj_body(c, carry):
        c0 = pl.multiple_of(c * 512, 512)
        xc = x_v[pl.ds(c0, 512), :]
        r = lax.dot_general(wt_v[0:D + 64, :], xc, NT, preferred_element_type=F32)
        qt_v[:, pl.ds(c0, 512)] = _pack((r[0:D] * QSCALE).astype(BF))
        a_kv(c, r[D:D + 64])
        return carry

    lax.fori_loop(1, 4, a_proj_body, 0)

    for name in ("wqkv", "bx", "wob"):
        in_copy(name).start()

    NTA = H * (S // TQ)
    NJ = S // RK
    GA = 6
    NB = 3
    LAG = 2
    FSTEP = 4

    def a_qtile(t):
        h = t % H if isinstance(t, int) else lax.rem(t, H)
        qb = t // H
        if isinstance(t, int):
            return qt_v[h * 16:(h + 1) * 16, qb * TQ:(qb + 1) * TQ]
        return qt_v[pl.ds(pl.multiple_of(h * 16, 16), 16),
                    pl.ds(pl.multiple_of(qb * TQ, TQ), TQ)]

    def a_s1_round(qt, s_dst, j):
        kk = _unpack(ka_v[j * RK // 2:(j + 1) * RK // 2, :])
        s = jnp.dot(kk[:, 0:DH], qt, preferred_element_type=F32)
        s_dst[j * RK:(j + 1) * RK, :] = s
        return _red8(s, jnp.maximum)

    def a_s2_round(s_src, j, mb):
        s = s_src[j * RK:(j + 1) * RK, :]
        p = jnp.exp2(s.reshape(RK // 8, 8, TQ) - mb[None]).reshape(RK, TQ)
        lj = _red8(p, jnp.add)
        vt = _unpack(vta_v[:, j * RK:(j + 1) * RK])
        pv = jnp.dot(vt, p.astype(BF), preferred_element_type=F32)
        return lj, pv

    def a_block(n0, z, nslots=GA, with_s1=True, fillers=()):
        fillers = list(fillers)
        zv = jnp.full((8, TQ), z, jnp.int32).astype(U32)
        ms = [m_v[0:8, :], m_v[8:16, :]]
        hist = []
        for g in range(nslots):
            n = n0 + g
            if with_s1:
                qt = _unpack(a_qtile(n + 2))
            s_src = s_bufs[g % NB]
            s_dst = s_bufs[(g + 2) % NB]
            mb = ms[g]
            m = l = acc = None
            for j in range(NJ):
                if with_s1:
                    mj = a_s1_round(qt, s_dst, j)
                    m = mj if m is None else jnp.maximum(m, mj)
                    hist.append(m)
                w = g * NJ + j
                y = hist[w - LAG - 1] if (with_s1 and w - LAG - 1 >= 0) else None
                lj, pv = a_s2_round(s_src, j, _dep(mb, y, zv))
                l = lj if l is None else l + lj
                acc = pv if acc is None else acc + pv
                if fillers and j % FSTEP == 0:
                    fillers.pop(0)()
            if with_s1:
                ms.append(_colmax_b(m))
            l = jnp.sum(l, axis=0, keepdims=True)
            ota_v[(n >> 5) & 1, pl.ds(_off(n & (H - 1), DH, 0), DH), :] = (
                acc * (1.0 / l)).astype(BF)
        if with_s1:
            m_v[0:8, :] = ms[nslots]
            m_v[8:16, :] = ms[nslots + 1]

    OCH = 4

    def out_proj(ot_v, w_ref, slot, qb, half):
        n = 512 // OCH
        for c in range(OCH):
            ot = ot_v[:, c * n:(c + 1) * n]
            r = lax.dot_general(ot, w_ref[...], TN, preferred_element_type=F32)
            stage_v[slot, c * n:(c + 1) * n, :] = r.astype(BF)
            row0 = qb * 512 + c * n
            if not isinstance(qb, int):
                row0 = pl.multiple_of(row0, n)
            pltpu.make_async_copy(
                stage_v.at[slot, pl.ds(c * n, n)],
                out_hbm.at[pl.ds(row0, n), pl.ds(half * D, D)],
                out_sem.at[slot],
            ).start()

    def b_wt_chunk(c):
        c0 = _off(c, 512, 0) + (c // 2) * D
        if not isinstance(c, int):
            c0 = pl.multiple_of(c0, 512)
        wtb_v[pl.ds(_off(c, 512, 0), 512), :] = bwqkv_v[:, pl.ds(c0, 512)].T

    def a_out(qb):
        slot = qb & 1

        @pl.when(qb == 0)
        def _():
            in_copy("woa").wait()
            in_copy("wqkv").wait()

        @pl.when(qb == 2)
        def _():
            out_copy(0, 0, 0).wait()

        out_proj(ota_v.at[slot], wo_a, slot, qb, 0)
        b_wt_chunk(qb)

    for a in range(2):
        qt0 = _unpack(a_qtile(a))
        m0 = None
        for j in range(NJ):
            mj = a_s1_round(qt0, s_bufs[a], j)
            m0 = mj if m0 is None else jnp.maximum(m0, mj)
        m_v[a * 8:(a + 1) * 8, :] = _colmax_b(m0)

    NBLK = (NTA - 2) // GA
    assert NBLK * GA + 2 == NTA and GA % NB == 0

    def a_body(it, carry):
        z = it >> 16
        a_block(it * GA, z)
        qb = ((it + 1) * GA >> 5) - 1

        @pl.when((qb >= 0) & (qb < 3) & (qb == (it * GA >> 5)))
        def _():
            a_out(qb)
        return z

    z_last = lax.fori_loop(0, NBLK, a_body, 0)

    def b_q_piece(i, n):
        def f():
            r = lax.dot_general(wtb_v[i * n:(i + 1) * n, :], bx_v[0:512, :], NT,
                                preferred_element_type=F32)
            qt_v[i * n // 2:(i + 1) * n // 2, 0:512] = _pack((r * QSCALE).astype(BF))
        return f

    def b_proj_body(c, carry, with_q=True):
        c0 = _off(c, 512, 0)
        xc = bx_v[pl.ds(c0, 512), :]
        if with_q:
            r = lax.dot_general(wtb_v[0:D, :], xc, NT, preferred_element_type=F32)
            qt_v[:, pl.ds(c0, 512)] = _pack((r * QSCALE).astype(BF))
        r = lax.dot_general(wtb_v[D:2 * D, :], xc, NT, preferred_element_type=F32)
        vtb_v[:, pl.ds(c0, 512)] = _pack(r.astype(BF))
        r = jnp.dot(xc, bwqkv_v[:, D:2 * D], preferred_element_type=F32)
        kb_v[pl.ds(_off(c, 256, 0), 256), :] = _pack(r.astype(BF))
        return carry

    in_copy("bx").wait()
    b_wt_chunk(3)
    npiece = 2 * NJ // FSTEP
    a_block(NTA - 2, z_last, 2, False, [b_q_piece(i, D // npiece) for i in range(npiece)])
    b_proj_body(0, 0, with_q=False)
    lax.fori_loop(1, 4, b_proj_body, 0)

    ri = lax.broadcasted_iota(jnp.int32, (128, 128), 0)
    ci = lax.broadcasted_iota(jnp.int32, (128, 128), 1)
    NGRP = 8
    NTB = S // 128

    def rounds_of(t):
        return tuple(r for r in range(3) if t - 2 + r >= 0) if isinstance(t, int) else (0, 1, 2)

    def off(t, mul, add, mult):
        return t * mul + add if isinstance(t, int) else pl.multiple_of(t * mul + add, mult)

    class BU1:
        def __init__(self, t, g, s_dst, store_m):
            self.t, self.g, self.s_dst, self.store_m = t, g, s_dst, store_m
            q4 = qt_v[g * 64:(g + 1) * 64, pl.ds(off(t, 128, 0, 128), 128)]
            zz = jnp.zeros((16, 128), U32)
            ws = []
            for h in range(4):
                ws.append(jnp.concatenate(
                    [q4[hh * 16:(hh + 1) * 16] if hh == h else zz for hh in range(4)], axis=0))
            self.w = _unpack(jnp.concatenate(ws, axis=1))
            self.m = None

        def round(self, r):
            t, g = self.t, self.g
            kk = _unpack(kb_v[pl.ds(off(t, 64, (r - 2) * 64, 64), 64), g * 128:(g + 1) * 128])
            s = jnp.dot(kk, self.w, preferred_element_type=F32)
            if r != 1:
                valid = (ri > ci) if r == 0 else (ri <= ci)
                s = jnp.concatenate(
                    [jnp.where(valid, s[:, h * 128:(h + 1) * 128], NEG) for h in range(4)],
                    axis=1)
            self.s_dst[g * 384 + r * 128:g * 384 + (r + 1) * 128, :] = s
            mr = _red8(s, jnp.maximum)
            self.m = mr if self.m is None else jnp.maximum(self.m, mr)
            if r == 2 and self.store_m:
                m_v[g * 8:(g + 1) * 8, :] = self.m
            return mr

    class BU2:
        def __init__(self, t, oc, g, s_src, mb):
            self.t, self.oc, self.g, self.s_src, self.mb = t, oc, g, s_src, mb
            self.l = None
            self.accs = [None] * 4

        def round(self, r, y, zv):
            t, g = self.t, self.g
            s = self.s_src[g * 384 + r * 128:g * 384 + (r + 1) * 128, :]
            p = jnp.exp2(s.reshape(16, 8, 512) - _dep(self.mb, y, zv)[None]).reshape(128, 512)
            lr = _red8(p, jnp.add)
            self.l = lr if self.l is None else self.l + lr
            for h in range(4):
                pbh = p[:, h * 128:(h + 1) * 128].astype(BF)
                vt = _unpack(vtb_v[g * 64 + h * 16:g * 64 + (h + 1) * 16,
                                   pl.ds(off(t, 128, (r - 2) * 128, 128), 128)])
                pv = jnp.dot(vt, pbh, preferred_element_type=F32)
                self.accs[h] = pv if self.accs[h] is None else self.accs[h] + pv
            if r == 2:
                rl = 1.0 / jnp.sum(self.l, axis=0, keepdims=True)
                for h in range(4):
                    otb_v[g * 128 + h * DH:g * 128 + (h + 1) * DH, pl.ds(self.oc, 128)] = (
                        self.accs[h] * rl[:, h * 128:(h + 1) * 128]).astype(BF)

    r64 = lax.broadcasted_iota(jnp.int32, (64, 128), 0)
    c64 = lax.broadcasted_iota(jnp.int32, (64, 128), 1)
    jm = c64 & 63

    def valid_mask(k):
        if k < 4:
            j = (c64 + 64) & 127 if k % 2 else c64
            if k < 2:
                return j < r64 + 64
            return j >= r64
        return r64 > jm if k == 4 else r64 <= jm

    for k in range(6):
        cap_v[k * 64:(k + 1) * 64, :] = jnp.where(valid_mask(k), jnp.inf, NEG).astype(F32)

    def capped(x, k):
        return jnp.minimum(x, cap_v[k * 64:(k + 1) * 64, :])

    lane8 = lax.broadcasted_iota(jnp.int32, (8, 128), 1)
    keep_lo = jnp.where(lane8 < 64, -1, 0).astype(jnp.int32)
    keep_hi = jnp.where(lane8 < 64, 0, -1).astype(jnp.int32)

    def keep(x, low):
        n = x.shape[0] // 8
        xi = pltpu.bitcast(x, jnp.int32).reshape(n, 8, 128)
        xi = xi & (keep_lo if low else keep_hi)[None]
        return pltpu.bitcast(xi.reshape(n * 8, 128), x.dtype)

    def halves(a, b):
        lane = lax.broadcasted_iota(jnp.int32, a.shape, 1)
        return jnp.where(lane < 64, a, b)

    def tile(x, h):
        return x[:, h * 128:(h + 1) * 128]

    class BV1:
        def __init__(self, t, g, s_dst, store_m):
            self.t, self.g, self.s_dst, self.store_m = t, g, s_dst, store_m
            q4 = qt_v[g * 64:(g + 1) * 64, pl.ds(off(t, 128, 0, 128), 128)]
            qh = [q4[h * 16:(h + 1) * 16] for h in range(4)]
            qh = [pltpu.roll(q, 64, 1) if h % 2 else q for h, q in enumerate(qh)]
            zz = jnp.zeros((16, 128), U32)
            ws = [jnp.concatenate([qh[hh] if hh == h else zz for hh in range(4)], axis=0)
                  for h in range(4)]
            self.w = _unpack(jnp.concatenate(ws, axis=1))
            lo, hi = [], []
            for p in range(2):
                a, b = qh[2 * p], qh[2 * p + 1]
                pre, post = [zz] * (2 * p), [zz] * (2 - 2 * p)
                lo.append(jnp.concatenate(pre + [halves(a, zz), halves(zz, b)] + post, axis=0))
                hi.append(jnp.concatenate(pre + [halves(zz, a), halves(b, zz)] + post, axis=0))
            self.wlo = _unpack(jnp.concatenate(lo, axis=1))
            self.whi = _unpack(jnp.concatenate(hi, axis=1))
            self.m = None

        def keys(self, add, n):
            return _unpack(kb_v[pl.ds(off(self.t, 64, add // 2, 32), n // 2),
                                self.g * 128:(self.g + 1) * 128])

        def band(self, r):
            g = self.g
            s = jnp.dot(self.keys(-192 + 128 * r, 128), self.w,
                        preferred_element_type=F32)
            cols = []
            for h in range(4):
                top, bot = tile(s, h)[0:64], tile(s, h)[64:128]
                if r == 0:
                    top = capped(top, h % 2)
                else:
                    bot = capped(bot, 2 + h % 2)
                cols.append(jnp.concatenate([top, bot], axis=0))
            s = jnp.concatenate(cols, axis=1)
            self.s_dst[g * 384 + r * 128:g * 384 + (r + 1) * 128, :] = s
            return _red8(s, jnp.maximum)

        def edge(self, hi):
            g = self.g
            s = jnp.dot(self.keys(64 if hi else -256, 64), self.whi if hi else self.wlo,
                        preferred_element_type=F32)
            s = jnp.concatenate([capped(tile(s, p), 4 + hi) for p in range(2)], axis=1)
            self.s_dst[g * 384 + 256:g * 384 + 320, hi * 256:(hi + 1) * 256] = s
            mx = _red8(s, jnp.maximum)
            neg = jnp.full((8, 128), NEG, F32)
            return jnp.concatenate(
                [halves(tile(mx, h // 2), neg) if (h % 2) == hi else halves(neg, tile(mx, h // 2))
                 for h in range(4)], axis=1)

        def round(self, r):
            mr = self.band(r) if r < 2 else jnp.maximum(self.edge(0), self.edge(1))
            self.m = mr if self.m is None else jnp.maximum(self.m, mr)
            if r == 2 and self.store_m:
                m_v[self.g * 8:(self.g + 1) * 8, :] = self.m
            return mr

    class BV2:
        def __init__(self, t, oc, g, s_src, mb):
            self.t, self.oc, self.g, self.s_src, self.mb = t, oc, g, s_src, mb
            self.l = None
            self.accs = [None] * 4

        def probs(self, row0, n, mb):
            s = self.s_src[self.g * 384 + row0:self.g * 384 + row0 + n, :]
            return jnp.exp2(s.reshape(n // 8, 8, 512) - mb[None]).reshape(n, 512)

        def half_probs(self, col0, mb, swap):
            s = self.s_src[self.g * 384 + 256:self.g * 384 + 320, col0:col0 + 256]
            mm = jnp.concatenate(
                [halves(tile(mb, 2 * p + swap), tile(mb, 2 * p + 1 - swap)) for p in range(2)],
                axis=1)
            p = jnp.exp2(s.reshape(8, 8, 256) - mm[None]).reshape(64, 256)
            return [keep(tile(p, h // 2), (h % 2) == swap) for h in range(4)]

        def round(self, r, y, zv):
            t, g = self.t, self.g
            mb = _dep(self.mb, y, zv)
            if r == 0:
                top = self.half_probs(0, mb, 0)
                bot = self.probs(0, 64, mb)
                ps = [jnp.concatenate([top[h], tile(bot, h)], axis=0) for h in range(4)]
            elif r == 1:
                p = self.probs(64, 128, mb)
                ps = [tile(p, h) for h in range(4)]
            else:
                top = self.probs(192, 64, mb)
                bot = self.half_probs(256, mb, 1)
                ps = [jnp.concatenate([tile(top, h), bot[h]], axis=0) for h in range(4)]
            lr = jnp.concatenate([_red8(p, jnp.add) for p in ps], axis=1)
            self.l = lr if self.l is None else self.l + lr
            for h in range(4):
                vt = _unpack(vtb_v[g * 64 + h * 16:g * 64 + (h + 1) * 16,
                                   pl.ds(off(t, 128, (r - 2) * 128, 128), 128)])
                pv = jnp.dot(vt, ps[h].astype(BF), preferred_element_type=F32)
                self.accs[h] = pv if self.accs[h] is None else self.accs[h] + pv
            if r == 2:
                rl = 1.0 / jnp.sum(self.l, axis=0, keepdims=True)
                for h in range(4):
                    o = self.accs[h] * tile(rl, h)
                    if h % 2:
                        o = pltpu.roll(o, 64, 1)
                    otb_v[g * 128 + h * DH:g * 128 + (h + 1) * DH, pl.ds(self.oc, 128)] = (
                        o.astype(BF))

    def banded(t):
        return not (isinstance(t, int) and t < 2)

    BLAG = 2

    def b_block(slots, z):
        zv = jnp.full((8, 512), z, jnp.int32).astype(U32)
        hist = []
        mbs = None
        for si, (t, tn, s_src, s_dst) in enumerate(slots):
            if t is not None:
                if mbs is None:
                    mbs = [_colmax_b(m_v[g * 8:(g + 1) * 8, :]) for g in range(NGRP)]
                oc = ((t % 4) * 128 if isinstance(t, int)
                      else pl.multiple_of(lax.rem(t, 4) * 128, 128))
            nxt = []
            for g in range(NGRP):
                b = a = None
                if t is not None:
                    b = (BV2 if banded(t) else BU2)(t, oc, g, s_src, mbs[g])
                if tn is not None:
                    a = (BV1 if banded(tn) else BU1)(tn, g, s_dst, si == len(slots) - 1)
                for r in range(3):
                    w = len(hist)
                    if a is not None and r in rounds_of(tn):
                        hist.append(a.round(r))
                    else:
                        hist.append(None)
                    if b is not None and r in rounds_of(t):
                        y = hist[w - BLAG - 1] if w - BLAG - 1 >= 0 else None
                        b.round(r, y, zv)
                if a is not None:
                    nxt.append(a.m)
            mbs = [_colmax_b(m) for m in nxt] if (nxt and si < len(slots) - 1) else None

    def b_out(qb):
        slot = (qb + 1) & 1
        out_copy(slot, jnp.where(qb < 2, qb + 1, 0), jnp.where(qb < 2, 0, 1)).wait()
        out_proj(otb_v, wo_b, slot, qb, 1)

    b_block([(None, 0, None, s_0), (0, 1, s_0, s_1), (1, 2, s_1, s_0)], z_last)

    in_copy("wob").wait()

    def b_body(i, carry):
        t = 2 * i
        b_block([(t, t + 1, s_0, s_1), (t + 1, t + 2, s_1, s_0)], i >> 16)

        @pl.when((i & 1) == 1)
        def _():
            b_out(i >> 1)
        return carry

    lax.fori_loop(1, NTB // 2 - 1, b_body, 0)
    out_copy(0, 1, 1).wait()
    b_block([(NTB - 2, NTB - 1, s_0, s_1), (NTB - 1, None, s_1, None)], z_last)
    out_proj(ota_v.at[1], wo_a, 0, 3, 0)
    out_copy(1, 2, 1).wait()
    out_proj(otb_v, wo_b, 1, 3, 1)
    out_copy(0, 3, 0).wait()
    out_copy(1, 3, 1).wait()


@jax.jit
def pallas_concat_heads__grouped_kv_mqa__sliding_block__prompt_kernel(
    A_x: jax.Array,
    A_wq: jax.Array,
    A_wk: jax.Array,
    A_wv: jax.Array,
    A_wo: jax.Array,
    B_x: jax.Array,
    B_wqkv: jax.Array,
    B_wo: jax.Array,
):
    B = A_x.shape[0]
    assert B == 1 and A_x.shape == (1, S, D) and B_x.shape == (1, S, D)

    scratch = [
        pltpu.VMEM((S, D), BF),
        pltpu.VMEM((D, D), BF),
        pltpu.VMEM((D, D), BF),
        pltpu.VMEM((S, D), BF),
        pltpu.VMEM((D, 3 * D), BF),
        pltpu.VMEM((D, D), BF),
        pltpu.VMEM((D + 64, D), BF),
        pltpu.VMEM((2 * D, D), BF),
        pltpu.VMEM((D // 2, S), U32),
        pltpu.VMEM((S // 2, 128), U32),
        pltpu.VMEM((DH // 2, S), U32),
        pltpu.VMEM((S // 2, D), U32),
        pltpu.VMEM((D // 2, S), U32),
        pltpu.VMEM((2, D, 512), BF),
        pltpu.VMEM((D, 512), BF),
        pltpu.VMEM((2, 512, D), BF),
        pltpu.VMEM((64, 512), F32),
        pltpu.VMEM((6 * 64, 128), F32),
        pltpu.VMEM((SROWS, 512), F32),
        pltpu.VMEM((SROWS, 512), F32),
        pltpu.VMEM((S, 512), F32),
        pltpu.SemaphoreType.DMA((14,)),
        pltpu.SemaphoreType.DMA((2,)),
    ]
    any_spec = pl.BlockSpec(memory_space=pl.ANY)
    out = pl.pallas_call(
        _kernel,
        out_shape=jax.ShapeDtypeStruct((S, 2 * D), BF),
        in_specs=[any_spec] * 8,
        out_specs=any_spec,
        scratch_shapes=scratch,
        compiler_params=pltpu.CompilerParams(vmem_limit_bytes=120 * 1024 * 1024),
    )(A_x.reshape(S, D), A_wq, A_wk.T, A_wv.T, A_wo, B_x.reshape(S, D), B_wqkv, B_wo)
    return out.reshape(1, S, 2 * D)
```

```python
import jax
import jax.numpy as jnp
from jax import lax
import jax.experimental.pallas as pl
import jax.experimental.pallas.tpu as pltpu


S = 2048
D = 1024
H = 32
DH = D // H
W = 256
LOG2E = 1.4426950408889634
QSCALE = (DH ** -0.5) * LOG2E
NEG = -1e9 * LOG2E

TQ = 512
RK = 128
SROWS = 3 * 128 * 8
assert W == 256

BF = jnp.bfloat16
U32 = jnp.uint32
F32 = jnp.float32
NT = (((1,), (1,)), ((), ()))
TN = (((0,), (0,)), ((), ()))


def _tree(xs, op):
    xs = list(xs)
    while len(xs) > 1:
        nx = [op(xs[i], xs[i + 1]) for i in range(0, len(xs) - 1, 2)]
        if len(xs) % 2:
            nx.append(xs[-1])
        xs = nx
    return xs[0]


def _red8(x, op):
    n = x.shape[0] // 8
    x = x.reshape(n, 8, x.shape[1])
    return _tree([x[i] for i in range(n)], op)


def _pack(x_bf16):
    return pltpu.bitcast(x_bf16, U32)


def _unpack(x_u32):
    return pltpu.bitcast(x_u32, BF)


def _dep(x, y, zv):
    if y is None:
        return x
    xb = pltpu.bitcast(x, U32)
    yb = pltpu.bitcast(y, U32)
    return pltpu.bitcast(xb | (yb & zv), x.dtype)


def _off(i, mul, add):
    return i * mul + add if isinstance(i, int) else pl.multiple_of(i * mul + add, mul)


def _colmax_b(m):
    return jnp.broadcast_to(jnp.max(m, axis=0, keepdims=True), m.shape)


def _kernel(
    ax_hbm, awq_hbm, awk_hbm, awv_hbm, awo_hbm, bx_hbm, bwqkv_hbm, bwo_hbm,
    out_hbm,
    x_v, wq_v, wo_a, bx_v, bwqkv_v, wo_b,
    wt_v, wtb_v, qt_v, ka_v, vta_v, kb_v, vtb_v, ota_v, otb_v, stage_v, m_v, cap_v,
    s_0, s_1, s_2,
    in_sem, out_sem,
):
    s_bufs = (s_0, s_1, s_2)

    IN = {}
    for c in range(4):
        IN["wq%d" % c] = (awq_hbm.at[:, pl.ds(c * 256, 256)], wq_v.at[:, pl.ds(c * 256, 256)])
        IN["x%d" % c] = (ax_hbm.at[pl.ds(c * 512, 512)], x_v.at[pl.ds(c * 512, 512)])
    IN["wk"] = (awk_hbm, wt_v.at[pl.ds(0, DH)])
    IN["wv"] = (awv_hbm, wt_v.at[pl.ds(DH, DH)])
    IN["woa"] = (awo_hbm, wo_a)
    IN["wqkv"] = (bwqkv_hbm, bwqkv_v)
    IN["bx"] = (bx_hbm, bx_v)
    IN["wob"] = (bwo_hbm, wo_b)
    IN_IDX = {k: i for i, k in enumerate(sorted(IN))}

    def in_copy(name):
        src, dst = IN[name]
        return pltpu.make_async_copy(src, dst, in_sem.at[IN_IDX[name]])

    def out_copy(slot, qb, half):
        return pltpu.make_async_copy(
            stage_v.at[slot],
            out_hbm.at[pl.ds(_off(qb, 512, 0), 512), pl.ds(_off(half, D, 0), D)],
            out_sem.at[slot],
        )

    for name in ("wq0", "wk", "wv", "x0"):
        in_copy(name).start()

    KV = 2 * DH

    def a_kv(c, r):
        kv = jnp.concatenate([r, jnp.zeros((128 - KV, 512), F32)], axis=0)
        ka_v[pl.ds(_off(c, 256, 0), 256), :] = _pack(kv.T.astype(BF))
        vta_v[:, pl.ds(_off(c, 512, 0), 512)] = _pack(r[DH:KV].astype(BF))

    in_copy("wq0").wait()
    for name in ("wq1", "wq2", "wq3"):
        in_copy(name).start()
    wt_v[KV:KV + 256, :] = wq_v[:, 0:256].T
    in_copy("wk").wait()
    in_copy("wv").wait()
    in_copy("x0").wait()
    for name in ("x1", "x2", "x3", "woa"):
        in_copy(name).start()
    xc = x_v[0:512, :]
    r = lax.dot_general(wt_v[0:KV + 256, :], xc, NT, preferred_element_type=F32)
    a_kv(0, r[0:KV])
    qt_v[0:128, 0:512] = _pack((r[KV:] * QSCALE).astype(BF))
    for c in range(1, 4):
        in_copy("wq%d" % c).wait()
    for c in range(1, 4):
        wt_v[KV + c * 256:KV + (c + 1) * 256, :] = wq_v[:, c * 256:(c + 1) * 256].T
    for c in range(1, 4):
        r = lax.dot_general(wt_v[KV + c * 256:KV + (c + 1) * 256, :], xc, NT,
                            preferred_element_type=F32)
        qt_v[c * 128:(c + 1) * 128, 0:512] = _pack((r * QSCALE).astype(BF))
    for c in range(1, 4):
        in_copy("x%d" % c).wait()

    def a_proj_body(c, carry):
        c0 = pl.multiple_of(c * 512, 512)
        xc = x_v[pl.ds(c0, 512), :]
        r = lax.dot_general(wt_v[0:D + 64, :], xc, NT, preferred_element_type=F32)
        a_kv(c, r[0:KV])
        qt_v[:, pl.ds(c0, 512)] = _pack((r[KV:] * QSCALE).astype(BF))
        return carry

    lax.fori_loop(1, 4, a_proj_body, 0)

    for name in ("wqkv", "bx", "wob"):
        in_copy(name).start()

    NTA = H * (S // TQ)
    NJ = S // RK
    GA = 6
    NB = 3
    LAG = 2
    FSTEP = 4

    def a_qtile(t):
        h = t % H if isinstance(t, int) else lax.rem(t, H)
        qb = t // H
        if isinstance(t, int):
            return qt_v[h * 16:(h + 1) * 16, qb * TQ:(qb + 1) * TQ]
        return qt_v[pl.ds(pl.multiple_of(h * 16, 16), 16),
                    pl.ds(pl.multiple_of(qb * TQ, TQ), TQ)]

    def a_s1_round(qt, s_dst, j):
        kk = _unpack(ka_v[j * RK // 2:(j + 1) * RK // 2, :])
        s = jnp.dot(kk[:, 0:DH], qt, preferred_element_type=F32)
        s_dst[j * RK:(j + 1) * RK, :] = s
        return _red8(s, jnp.maximum)

    def a_s2_round(s_src, j, mb):
        s = s_src[j * RK:(j + 1) * RK, :]
        p = jnp.exp2(s.reshape(RK // 8, 8, TQ) - mb[None]).reshape(RK, TQ)
        lj = _red8(p, jnp.add)
        vt = _unpack(vta_v[:, j * RK:(j + 1) * RK])
        pv = jnp.dot(vt, p.astype(BF), preferred_element_type=F32)
        return lj, pv

    def a_block(n0, z, nslots=GA, with_s1=True, fillers=()):
        fillers = list(fillers)
        zv = jnp.full((8, TQ), z, jnp.int32).astype(U32)
        ms = [m_v[0:8, :], m_v[8:16, :]]
        hist = []
        for g in range(nslots):
            n = n0 + g
            if with_s1:
                qt = _unpack(a_qtile(n + 2))
            s_src = s_bufs[g % NB]
            s_dst = s_bufs[(g + 2) % NB]
            mb = ms[g]
            m = l = acc = None
            for j in range(NJ):
                if with_s1:
                    mj = a_s1_round(qt, s_dst, j)
                    m = mj if m is None else jnp.maximum(m, mj)
                    hist.append(m)
                w = g * NJ + j
                y = hist[w - LAG - 1] if (with_s1 and w - LAG - 1 >= 0) else None
                lj, pv = a_s2_round(s_src, j, _dep(mb, y, zv))
                l = lj if l is None else l + lj
                acc = pv if acc is None else acc + pv
                if fillers and j % FSTEP == 0:
                    fillers.pop(0)()
            if with_s1:
                ms.append(_colmax_b(m))
            l = jnp.sum(l, axis=0, keepdims=True)
            ota_v[(n >> 5) & 1, pl.ds(_off(n & (H - 1), DH, 0), DH), :] = (
                acc * (1.0 / l)).astype(BF)
        if with_s1:
            m_v[0:8, :] = ms[nslots]
            m_v[8:16, :] = ms[nslots + 1]

    OCH = 4

    def out_proj(ot_v, w_ref, slot, qb, half):
        n = 512 // OCH
        for c in range(OCH):
            ot = ot_v[:, c * n:(c + 1) * n]
            r = lax.dot_general(ot, w_ref[...], TN, preferred_element_type=F32)
            stage_v[slot, c * n:(c + 1) * n, :] = r.astype(BF)
            row0 = qb * 512 + c * n
            if not isinstance(qb, int):
                row0 = pl.multiple_of(row0, n)
            pltpu.make_async_copy(
                stage_v.at[slot, pl.ds(c * n, n)],
                out_hbm.at[pl.ds(row0, n), pl.ds(half * D, D)],
                out_sem.at[slot],
            ).start()

    def b_wt_chunk(c):
        c0 = _off(c, 512, 0) + (c // 2) * D
        if not isinstance(c, int):
            c0 = pl.multiple_of(c0, 512)
        wtb_v[pl.ds(_off(c, 512, 0), 512), :] = bwqkv_v[:, pl.ds(c0, 512)].T

    def a_out(qb):
        slot = qb & 1

        @pl.when(qb == 0)
        def _():
            in_copy("woa").wait()
            in_copy("wqkv").wait()

        @pl.when(qb == 2)
        def _():
            out_copy(0, 0, 0).wait()

        out_proj(ota_v.at[slot], wo_a, slot, qb, 0)
        b_wt_chunk(qb)

    for a in range(2):
        qt0 = _unpack(a_qtile(a))
        m0 = None
        for j in range(NJ):
            mj = a_s1_round(qt0, s_bufs[a], j)
            m0 = mj if m0 is None else jnp.maximum(m0, mj)
        m_v[a * 8:(a + 1) * 8, :] = _colmax_b(m0)

    NBLK = (NTA - 2) // GA
    assert NBLK * GA + 2 == NTA and GA % NB == 0

    def a_body(it, carry):
        z = it >> 16
        a_block(it * GA, z)
        qb = ((it + 1) * GA >> 5) - 1

        @pl.when((qb >= 0) & (qb < 3) & (qb == (it * GA >> 5)))
        def _():
            a_out(qb)
        return z

    z_last = lax.fori_loop(0, NBLK, a_body, 0)

    def b_q_piece(i, n):
        def f():
            r = lax.dot_general(wtb_v[i * n:(i + 1) * n, :], bx_v[0:512, :], NT,
                                preferred_element_type=F32)
            qt_v[i * n // 2:(i + 1) * n // 2, 0:512] = _pack((r * QSCALE).astype(BF))
        return f

    def b_proj_body(c, carry, with_q=True):
        c0 = _off(c, 512, 0)
        xc = bx_v[pl.ds(c0, 512), :]
        if with_q:
            r = lax.dot_general(wtb_v[0:D, :], xc, NT, preferred_element_type=F32)
            qt_v[:, pl.ds(c0, 512)] = _pack((r * QSCALE).astype(BF))
        r = lax.dot_general(wtb_v[D:2 * D, :], xc, NT, preferred_element_type=F32)
        vtb_v[:, pl.ds(c0, 512)] = _pack(r.astype(BF))
        r = jnp.dot(xc, bwqkv_v[:, D:2 * D], preferred_element_type=F32)
        kb_v[pl.ds(_off(c, 256, 0), 256), :] = _pack(r.astype(BF))
        return carry

    in_copy("bx").wait()
    b_wt_chunk(3)
    npiece = 2 * NJ // FSTEP
    a_block(NTA - 2, z_last, 2, False, [b_q_piece(i, D // npiece) for i in range(npiece)])
    b_proj_body(0, 0, with_q=False)
    lax.fori_loop(1, 4, b_proj_body, 0)

    ri = lax.broadcasted_iota(jnp.int32, (128, 128), 0)
    ci = lax.broadcasted_iota(jnp.int32, (128, 128), 1)
    NGRP = 8
    NTB = S // 128

    def rounds_of(t):
        return tuple(r for r in range(3) if t - 2 + r >= 0) if isinstance(t, int) else (0, 1, 2)

    def off(t, mul, add, mult):
        return t * mul + add if isinstance(t, int) else pl.multiple_of(t * mul + add, mult)

    class BU1:
        def __init__(self, t, g, s_dst, store_m):
            self.t, self.g, self.s_dst, self.store_m = t, g, s_dst, store_m
            q4 = qt_v[g * 64:(g + 1) * 64, pl.ds(off(t, 128, 0, 128), 128)]
            zz = jnp.zeros((16, 128), U32)
            ws = []
            for h in range(4):
                ws.append(jnp.concatenate(
                    [q4[hh * 16:(hh + 1) * 16] if hh == h else zz for hh in range(4)], axis=0))
            self.w = _unpack(jnp.concatenate(ws, axis=1))
            self.m = None

        def round(self, r):
            t, g = self.t, self.g
            kk = _unpack(kb_v[pl.ds(off(t, 64, (r - 2) * 64, 64), 64), g * 128:(g + 1) * 128])
            s = jnp.dot(kk, self.w, preferred_element_type=F32)
            if r != 1:
                valid = (ri > ci) if r == 0 else (ri <= ci)
                s = jnp.concatenate(
                    [jnp.where(valid, s[:, h * 128:(h + 1) * 128], NEG) for h in range(4)],
                    axis=1)
            self.s_dst[g * 384 + r * 128:g * 384 + (r + 1) * 128, :] = s
            mr = _red8(s, jnp.maximum)
            self.m = mr if self.m is None else jnp.maximum(self.m, mr)
            if r == 2 and self.store_m:
                m_v[g * 8:(g + 1) * 8, :] = self.m
            return mr

    class BU2:
        def __init__(self, t, oc, g, s_src, mb):
            self.t, self.oc, self.g, self.s_src, self.mb = t, oc, g, s_src, mb
            self.l = None
            self.accs = [None] * 4

        def round(self, r, y, zv):
            t, g = self.t, self.g
            s = self.s_src[g * 384 + r * 128:g * 384 + (r + 1) * 128, :]
            p = jnp.exp2(s.reshape(16, 8, 512) - _dep(self.mb, y, zv)[None]).reshape(128, 512)
            lr = _red8(p, jnp.add)
            self.l = lr if self.l is None else self.l + lr
            for h in range(4):
                pbh = p[:, h * 128:(h + 1) * 128].astype(BF)
                vt = _unpack(vtb_v[g * 64 + h * 16:g * 64 + (h + 1) * 16,
                                   pl.ds(off(t, 128, (r - 2) * 128, 128), 128)])
                pv = jnp.dot(vt, pbh, preferred_element_type=F32)
                self.accs[h] = pv if self.accs[h] is None else self.accs[h] + pv
            if r == 2:
                rl = 1.0 / jnp.sum(self.l, axis=0, keepdims=True)
                for h in range(4):
                    otb_v[g * 128 + h * DH:g * 128 + (h + 1) * DH, pl.ds(self.oc, 128)] = (
                        self.accs[h] * rl[:, h * 128:(h + 1) * 128]).astype(BF)

    r64 = lax.broadcasted_iota(jnp.int32, (64, 128), 0)
    c64 = lax.broadcasted_iota(jnp.int32, (64, 128), 1)
    jm = c64 & 63

    def valid_mask(k):
        if k < 4:
            j = (c64 + 64) & 127 if k % 2 else c64
            if k < 2:
                return j < r64 + 64
            return j >= r64
        return r64 > jm if k == 4 else r64 <= jm

    for k in range(6):
        cap_v[k * 64:(k + 1) * 64, :] = jnp.where(valid_mask(k), jnp.inf, NEG).astype(F32)

    def capped(x, k):
        return jnp.minimum(x, cap_v[k * 64:(k + 1) * 64, :])

    lane8 = lax.broadcasted_iota(jnp.int32, (8, 128), 1)
    keep_lo = jnp.where(lane8 < 64, -1, 0).astype(jnp.int32)
    keep_hi = jnp.where(lane8 < 64, 0, -1).astype(jnp.int32)

    def keep(x, low):
        n = x.shape[0] // 8
        xi = pltpu.bitcast(x, jnp.int32).reshape(n, 8, 128)
        xi = xi & (keep_lo if low else keep_hi)[None]
        return pltpu.bitcast(xi.reshape(n * 8, 128), x.dtype)

    def halves(a, b):
        lane = lax.broadcasted_iota(jnp.int32, a.shape, 1)
        return jnp.where(lane < 64, a, b)

    def tile(x, h):
        return x[:, h * 128:(h + 1) * 128]

    class BV1:
        def __init__(self, t, g, s_dst, store_m):
            self.t, self.g, self.s_dst, self.store_m = t, g, s_dst, store_m
            q4 = qt_v[g * 64:(g + 1) * 64, pl.ds(off(t, 128, 0, 128), 128)]
            qh = [q4[h * 16:(h + 1) * 16] for h in range(4)]
            qh = [pltpu.roll(q, 64, 1) if h % 2 else q for h, q in enumerate(qh)]
            zz = jnp.zeros((16, 128), U32)
            ws = [jnp.concatenate([qh[hh] if hh == h else zz for hh in range(4)], axis=0)
                  for h in range(4)]
            self.w = _unpack(jnp.concatenate(ws, axis=1))
            lo, hi = [], []
            for p in range(2):
                a, b = qh[2 * p], qh[2 * p + 1]
                pre, post = [zz] * (2 * p), [zz] * (2 - 2 * p)
                lo.append(jnp.concatenate(pre + [halves(a, zz), halves(zz, b)] + post, axis=0))
                hi.append(jnp.concatenate(pre + [halves(zz, a), halves(b, zz)] + post, axis=0))
            self.wlo = _unpack(jnp.concatenate(lo, axis=1))
            self.whi = _unpack(jnp.concatenate(hi, axis=1))
            self.m = None

        def keys(self, add, n):
            return _unpack(kb_v[pl.ds(off(self.t, 64, add // 2, 32), n // 2),
                                self.g * 128:(self.g + 1) * 128])

        def band(self, r):
            g = self.g
            s = jnp.dot(self.keys(-192 + 128 * r, 128), self.w,
                        preferred_element_type=F32)
            cols = []
            for h in range(4):
                top, bot = tile(s, h)[0:64], tile(s, h)[64:128]
                if r == 0:
                    top = capped(top, h % 2)
                else:
                    bot = capped(bot, 2 + h % 2)
                cols.append(jnp.concatenate([top, bot], axis=0))
            s = jnp.concatenate(cols, axis=1)
            self.s_dst[g * 384 + r * 128:g * 384 + (r + 1) * 128, :] = s
            return _red8(s, jnp.maximum)

        def edge(self, hi):
            g = self.g
            s = jnp.dot(self.keys(64 if hi else -256, 64), self.whi if hi else self.wlo,
                        preferred_element_type=F32)
            s = jnp.concatenate([capped(tile(s, p), 4 + hi) for p in range(2)], axis=1)
            self.s_dst[g * 384 + 256:g * 384 + 320, hi * 256:(hi + 1) * 256] = s
            mx = _red8(s, jnp.maximum)
            neg = jnp.full((8, 128), NEG, F32)
            return jnp.concatenate(
                [halves(tile(mx, h // 2), neg) if (h % 2) == hi else halves(neg, tile(mx, h // 2))
                 for h in range(4)], axis=1)

        def round(self, r):
            mr = self.band(r) if r < 2 else jnp.maximum(self.edge(0), self.edge(1))
            self.m = mr if self.m is None else jnp.maximum(self.m, mr)
            if r == 2 and self.store_m:
                m_v[self.g * 8:(self.g + 1) * 8, :] = self.m
            return mr

    class BV2:
        def __init__(self, t, oc, g, s_src, mb):
            self.t, self.oc, self.g, self.s_src, self.mb = t, oc, g, s_src, mb
            self.l = None
            self.accs = [None] * 4

        def probs(self, row0, n, mb):
            s = self.s_src[self.g * 384 + row0:self.g * 384 + row0 + n, :]
            return jnp.exp2(s.reshape(n // 8, 8, 512) - mb[None]).reshape(n, 512)

        def half_probs(self, col0, mb, swap):
            s = self.s_src[self.g * 384 + 256:self.g * 384 + 320, col0:col0 + 256]
            mm = jnp.concatenate(
                [halves(tile(mb, 2 * p + swap), tile(mb, 2 * p + 1 - swap)) for p in range(2)],
                axis=1)
            p = jnp.exp2(s.reshape(8, 8, 256) - mm[None]).reshape(64, 256)
            return [keep(tile(p, h // 2), (h % 2) == swap) for h in range(4)]

        def round(self, r, y, zv):
            t, g = self.t, self.g
            mb = _dep(self.mb, y, zv)
            if r == 0:
                top = self.half_probs(0, mb, 0)
                bot = self.probs(0, 64, mb)
                ps = [jnp.concatenate([top[h], tile(bot, h)], axis=0) for h in range(4)]
            elif r == 1:
                p = self.probs(64, 128, mb)
                ps = [tile(p, h) for h in range(4)]
            else:
                top = self.probs(192, 64, mb)
                bot = self.half_probs(256, mb, 1)
                ps = [jnp.concatenate([tile(top, h), bot[h]], axis=0) for h in range(4)]
            lr = jnp.concatenate([_red8(p, jnp.add) for p in ps], axis=1)
            self.l = lr if self.l is None else self.l + lr
            for h in range(4):
                vt = _unpack(vtb_v[g * 64 + h * 16:g * 64 + (h + 1) * 16,
                                   pl.ds(off(t, 128, (r - 2) * 128, 128), 128)])
                pv = jnp.dot(vt, ps[h].astype(BF), preferred_element_type=F32)
                self.accs[h] = pv if self.accs[h] is None else self.accs[h] + pv
            if r == 2:
                rl = 1.0 / jnp.sum(self.l, axis=0, keepdims=True)
                for h in range(4):
                    o = self.accs[h] * tile(rl, h)
                    if h % 2:
                        o = pltpu.roll(o, 64, 1)
                    otb_v[g * 128 + h * DH:g * 128 + (h + 1) * DH, pl.ds(self.oc, 128)] = (
                        o.astype(BF))

    def banded(t):
        return not (isinstance(t, int) and t < 2)

    BLAG = 2

    def b_block(slots, z):
        zv = jnp.full((8, 512), z, jnp.int32).astype(U32)
        hist = []
        mbs = None
        for si, (t, tn, s_src, s_dst) in enumerate(slots):
            if t is not None:
                if mbs is None:
                    mbs = [_colmax_b(m_v[g * 8:(g + 1) * 8, :]) for g in range(NGRP)]
                oc = ((t % 4) * 128 if isinstance(t, int)
                      else pl.multiple_of(lax.rem(t, 4) * 128, 128))
            nxt = []
            for g in range(NGRP):
                b = a = None
                if t is not None:
                    b = (BV2 if banded(t) else BU2)(t, oc, g, s_src, mbs[g])
                if tn is not None:
                    a = (BV1 if banded(tn) else BU1)(tn, g, s_dst, si == len(slots) - 1)
                for r in range(3):
                    w = len(hist)
                    if a is not None and r in rounds_of(tn):
                        hist.append(a.round(r))
                    else:
                        hist.append(None)
                    if b is not None and r in rounds_of(t):
                        y = hist[w - BLAG - 1] if w - BLAG - 1 >= 0 else None
                        b.round(r, y, zv)
                if a is not None:
                    nxt.append(a.m)
            mbs = [_colmax_b(m) for m in nxt] if (nxt and si < len(slots) - 1) else None

    def b_out(qb):
        slot = (qb + 1) & 1
        out_copy(slot, jnp.where(qb < 2, qb + 1, 0), jnp.where(qb < 2, 0, 1)).wait()
        out_proj(otb_v, wo_b, slot, qb, 1)

    b_block([(None, 0, None, s_0), (0, 1, s_0, s_1), (1, 2, s_1, s_0)], z_last)

    in_copy("wob").wait()

    def b_body(i, carry):
        t = 2 * i
        b_block([(t, t + 1, s_0, s_1), (t + 1, t + 2, s_1, s_0)], i >> 16)

        @pl.when((i & 1) == 1)
        def _():
            b_out(i >> 1)
        return carry

    lax.fori_loop(1, NTB // 2 - 1, b_body, 0)
    out_copy(0, 1, 1).wait()
    b_block([(NTB - 2, NTB - 1, s_0, s_1), (NTB - 1, None, s_1, None)], z_last)
    out_proj(ota_v.at[1], wo_a, 0, 3, 0)
    out_copy(1, 2, 1).wait()
    out_proj(otb_v, wo_b, 1, 3, 1)
    out_copy(0, 3, 0).wait()
    out_copy(1, 3, 1).wait()


@jax.jit
def pallas_concat_heads__grouped_kv_mqa__sliding_block__prompt_kernel(
    A_x: jax.Array,
    A_wq: jax.Array,
    A_wk: jax.Array,
    A_wv: jax.Array,
    A_wo: jax.Array,
    B_x: jax.Array,
    B_wqkv: jax.Array,
    B_wo: jax.Array,
):
    B = A_x.shape[0]
    assert B == 1 and A_x.shape == (1, S, D) and B_x.shape == (1, S, D)

    scratch = [
        pltpu.VMEM((S, D), BF),
        pltpu.VMEM((D, D), BF),
        pltpu.VMEM((D, D), BF),
        pltpu.VMEM((S, D), BF),
        pltpu.VMEM((D, 3 * D), BF),
        pltpu.VMEM((D, D), BF),
        pltpu.VMEM((D + 64, D), BF),
        pltpu.VMEM((2 * D, D), BF),
        pltpu.VMEM((D // 2, S), U32),
        pltpu.VMEM((S // 2, 128), U32),
        pltpu.VMEM((DH // 2, S), U32),
        pltpu.VMEM((S // 2, D), U32),
        pltpu.VMEM((D // 2, S), U32),
        pltpu.VMEM((2, D, 512), BF),
        pltpu.VMEM((D, 512), BF),
        pltpu.VMEM((2, 512, D), BF),
        pltpu.VMEM((64, 512), F32),
        pltpu.VMEM((6 * 64, 128), F32),
        pltpu.VMEM((SROWS, 512), F32),
        pltpu.VMEM((SROWS, 512), F32),
        pltpu.VMEM((S, 512), F32),
        pltpu.SemaphoreType.DMA((14,)),
        pltpu.SemaphoreType.DMA((2,)),
    ]
    any_spec = pl.BlockSpec(memory_space=pl.ANY)
    out = pl.pallas_call(
        _kernel,
        out_shape=jax.ShapeDtypeStruct((S, 2 * D), BF),
        in_specs=[any_spec] * 8,
        out_specs=any_spec,
        scratch_shapes=scratch,
        compiler_params=pltpu.CompilerParams(vmem_limit_bytes=96 * 1024 * 1024),
    )(A_x.reshape(S, D), A_wq, A_wk.T, A_wv.T, A_wo, B_x.reshape(S, D), B_wqkv, B_wo)
    return out.reshape(1, S, 2 * D)
```
